```python
import os as _os
_os.environ.setdefault("JAX_PLATFORMS", "cpu")
import jax
import jax.numpy as jnp

def _softmax(x, axis=-1):
    return jax.nn.softmax(x, axis=axis)
def _gelu(x):
    return jax.nn.gelu(x, approximate=True)
def _silu(x):
    return jax.nn.silu(x)
def _sigmoid(x):
    return jax.nn.sigmoid(x)
def _layernorm(x, axis=-1, eps=1e-5):
    m = jnp.mean(x, axis=axis, keepdims=True)
    v = jnp.var(x, axis=axis, keepdims=True)
    return (x - m) / jnp.sqrt(v + eps)
def _scatter_add(tgt, idx, src, axis=0):
    return tgt.at[idx].add(src)
def _segment_sum(src, seg, n):
    return jax.ops.segment_sum(src, seg, n)
class _Rng:
    def __init__(self, key):
        self._k = key
    def _next(self):
        self._k, sub = jax.random.split(self._k)
        return sub
    def normal(self, shape):
        return jax.random.normal(self._next(), shape, dtype=jnp.bfloat16)
    def randint(self, lo, hi, shape):
        return jax.random.randint(self._next(), shape, lo, hi, dtype=jnp.int32)
    def uniform(self, shape, lo=0.0, hi=1.0):
        return jax.random.uniform(self._next(), shape, jnp.bfloat16, lo, hi)
    def permutation(self, n):
        return jax.random.permutation(self._next(), n)


kernel_name = 'gated_mix__mha_block__dense_activation_mish__prompt'

def setup_inputs():
    _rng = _Rng(jax.random.key(int.from_bytes(__import__("os").urandom(4), "little")))
    _w = (lambda a: (lambda t: t.astype(jnp.bfloat16) if jnp.issubdtype(t.dtype, jnp.floating) else t)(jnp.asarray(a)))
    def _A_setup():
        B, S, D, H = 1, 2048, 640, 32
        return {
            "x": _w((lambda *s: _rng.normal(s) * 0.05)(B, S, D)),
            "wqkv": _w((lambda *s: _rng.normal(s) * 0.2)(D, 3 * D)),
            "wo": _w((lambda *s: _rng.normal(s) * 0.05)(D, D)),
        }
    _A_in = _A_setup()

    def _B_setup():
        B, S, D, F = 1, 2048, 640, 1536
        return {
            "x": _w((lambda *s: _rng.normal(s) * 0.05)(B, S, D)),
            "w1": _w((lambda *s: _rng.normal(s) * 0.8)(D, F) * (D ** -0.5)),
            "b1": _w((lambda *s: _rng.normal(s) * 0.05)(F)),
            "w2": _w((lambda *s: _rng.normal(s) * 0.05)(F, D) * (F ** -0.5)),
        }
    _B_in = _B_setup()

    return {
        "A_x": _A_in["x"],
        "A_wqkv": _A_in["wqkv"],
        "A_wo": _A_in["wo"],
        "B_x": _B_in["x"],
        "B_w1": _B_in["w1"],
        "B_b1": _B_in["b1"],
        "B_w2": _B_in["w2"],
        "gate_w": _w((lambda *s: _rng.normal(s) * 0.05)(640) * 16.0),
    }

def reference(A_x, A_wqkv, A_wo, B_x, B_w1, B_b1, B_w2, gate_w):
    def _A_ref(x, wqkv, wo):
        B, S, D = x.shape
        H = 32
        Dh = D // H
        qkv = (lambda x, *d: x.transpose(*d))((x @ wqkv).reshape(B, S, 3, H, Dh), 2, 0, 3, 1, 4)
        q, k, v = qkv[0], qkv[1], qkv[2]
        scores = jnp.einsum("bhqd,bhkd->bhqk", q, k) * (Dh ** -0.5)
        p = _softmax(scores, axis=-1)
        o = jnp.einsum("bhqk,bhkd->bhqd", p, v)
        return (lambda x, *d: x.transpose(*d))(o, 0, 2, 1, 3).reshape(B, S, D) @ wo

    def _B_ref(x, w1, b1, w2):
        h = jnp.einsum("bsd,df->bsf", x, w1) + b1
        sp = jnp.log1p(jnp.exp(-jnp.abs(h))) + jnp.where(h > 0, h, jnp.zeros_like(h))
        act = h * jnp.tanh(sp)
        return jnp.einsum("bsf,fd->bsd", act, w2)

    x = A_x
    g = _sigmoid((x * gate_w).sum(-1, keepdims=True))
    a = _A_ref(x, A_wqkv, A_wo)
    b = _B_ref(x, B_w1, B_b1, B_w2)
    return g * a + (1 - g) * b
```

```python
import functools
import math

import jax
import jax.numpy as jnp
from jax import lax
import jax.experimental.pallas as pl
import jax.experimental.pallas.tpu as pltpu

bf16 = jnp.bfloat16
f32 = jnp.float32

S, D, H, DH, F = 2048, 640, 32, 20, 1536
HPT = 6
NT = (H + HPT - 1) // HPT
DP = NT * 128
GATE_LANE = HPT * DH
QSCALE = (DH ** -0.5) * math.log2(math.e)
L_LO, L_HI = 2.0 ** -60, 2.0 ** 60


def _pad_heads(w):
    parts = []
    for t in range(NT):
        lo = t * HPT * DH
        hi = min(lo + HPT * DH, D)
        parts.append(w[:, lo:hi])
        parts.append(jnp.zeros((w.shape[0], 128 - (hi - lo)), w.dtype))
    return jnp.concatenate(parts, axis=1)


def _mish(h):
    e = jnp.exp(jnp.minimum(h, 20.0))
    n = e * (e + 2.0)
    return h * (n / (n + 2.0))


def make_kernel(TQ=1024, KB=128, DEPTH=2, PB=512, FB=512, FC=512):
    NQ = S // TQ

    def kernel(x_ref, wqkv_ref, wo_ref, w1_ref, b1_ref, w2_ref, gw_ref, o_ref,
               wqvT_s, wk_s, k_s, qT_s, vT_s, oT_s, g_s):
        wq = _pad_heads(wqkv_ref[:, 0:D])
        wqvT_s[0:DP, :] = wq.T
        wqvT_s[DP:DP + D, :] = wqkv_ref[:, 2 * D:3 * D].T
        wk = _pad_heads(wqkv_ref[:, D:2 * D])
        gcol = jnp.broadcast_to(gw_ref[...], (128, D)).T
        lane = lax.broadcasted_iota(jnp.int32, (D, 128), 1)
        wk_s[:, 0:128] = jnp.where(lane == GATE_LANE, gcol, wk[:, 0:128])
        wk_s[:, 128:DP] = wk[:, 128:DP]

        def proj(i, _):
            r = pl.multiple_of(i * PB, PB)
            xb = x_ref[pl.ds(r, PB), :]
            qv = lax.dot_general(wqvT_s[...], xb, (((1,), (1,)), ((), ())),
                                 preferred_element_type=f32)
            qT_s[:, pl.ds(r, PB)] = (qv[0:DP] * QSCALE).astype(bf16)
            vT_s[:, pl.ds(r, PB)] = qv[DP:DP + D].astype(bf16).astype(f32)
            kk = jnp.dot(xb, wk_s[...], preferred_element_type=f32)
            k_s[pl.ds(r, PB), :] = kk.astype(bf16)
            g = jax.nn.sigmoid(kk[:, GATE_LANE:GATE_LANE + 1])
            g_s[pl.ds(r, PB), :] = jnp.broadcast_to(g, (PB, 128))
            return 0
        lax.fori_loop(0, S // PB, proj, 0)

        def head_setup(it):
            h = it // NQ
            qo = pl.multiple_of((it % NQ) * TQ, TQ)
            t = pl.multiple_of((h // HPT) * 128, 128)
            lo = (h % HPT) * DH
            q = qT_s[pl.ds(t, 128), pl.ds(qo, TQ)]
            ri = lax.broadcasted_iota(jnp.int32, (128, TQ), 0)
            q = jnp.where((ri >= lo) & (ri < lo + DH), q, jnp.zeros_like(q))
            odd = h % 2
            vo = pl.multiple_of((h // 2) * 40 + odd * 16, 8)
            wr = lax.broadcasted_iota(jnp.int32, (24, 128), 0)
            valid = (wr >= odd * 4) & (wr < odd * 4 + DH)
            return qo, t, q, vo, valid, odd

        def finish(acc, qo, vo, odd):
            wr = lax.broadcasted_iota(jnp.int32, (24, TQ), 0)
            valid = (wr >= odd * 4) & (wr < odd * 4 + DH)
            l = jnp.max(jnp.where(valid, 0.0, acc), axis=0, keepdims=True)
            o = acc / l
            old = oT_s[pl.ds(vo, 24), pl.ds(qo, TQ)]
            oT_s[pl.ds(vo, 24), pl.ds(qo, TQ)] = jnp.where(valid, o, old)
            return l

        oT_s[...] = jnp.zeros_like(oT_s)

        def attn_fast(it, bad):
            qo, t, q, vo, valid, odd = head_setup(it)
            n = S // KB
            ps = []
            acc = None

            def pv(i, acc):
                v = vT_s[pl.ds(vo, 24), i * KB:(i + 1) * KB]
                vm = jnp.tile(valid, (1, KB // 128)) if KB > 128 else valid
                v = jnp.where(vm, v, 1.0)
                d = lax.dot_general(v, ps[i], (((1,), (0,)), ((), ())),
                                    preferred_element_type=f32)
                return d if acc is None else acc + d
            for i in range(n):
                st = jnp.dot(k_s[i * KB:(i + 1) * KB, pl.ds(t, 128)], q,
                             preferred_element_type=f32)
                if i >= DEPTH:
                    acc = pv(i - DEPTH, acc)
                ps.append(jnp.exp2(st).astype(bf16))
            for i in range(n - DEPTH, n):
                acc = pv(i, acc)
            l = finish(acc, qo, vo, odd)
            ok = (l >= L_LO) & (l <= L_HI)
            return jnp.maximum(bad, jnp.where(ok, 0.0, 1.0))
        bad = lax.fori_loop(0, H * NQ, attn_fast, jnp.zeros((1, TQ), f32))

        @pl.when(jnp.max(bad) > 0.0)
        def _safe():
            SB = 256

            def attn_safe(it, _):
                qo, t, q, vo, valid, odd = head_setup(it)

                def mx(i, m):
                    r = pl.multiple_of(i * SB, SB)
                    st = jnp.dot(k_s[pl.ds(r, SB), pl.ds(t, 128)], q, preferred_element_type=f32)
                    return jnp.maximum(m, jnp.max(st, axis=0, keepdims=True))
                m = lax.fori_loop(0, S // SB, mx, jnp.full((1, TQ), -jnp.inf, f32))

                def ex(i, acc):
                    r = pl.multiple_of(i * SB, SB)
                    st = jnp.dot(k_s[pl.ds(r, SB), pl.ds(t, 128)], q, preferred_element_type=f32)
                    p = jnp.exp2(st - m).astype(bf16)
                    v = vT_s[pl.ds(vo, 24), pl.ds(r, SB)]
                    v = jnp.where(jnp.tile(valid, (1, SB // 128)), v, 1.0)
                    return acc + lax.dot_general(v, p, (((1,), (0,)), ((), ())),
                                                 preferred_element_type=f32)
                acc = lax.fori_loop(0, S // SB, ex, jnp.zeros((24, TQ), f32))
                finish(acc, qo, vo, odd)
                return 0
            lax.fori_loop(0, H * NQ, attn_safe, 0)

        def tail(i, _):
            r = pl.multiple_of(i * FB, FB)
            xb = x_ref[pl.ds(r, FB), :]
            ot = oT_s[:, pl.ds(r, FB)].astype(bf16)
            a = lax.dot_general(ot, wo_ref[...], (((0,), (0,)), ((), ())),
                                preferred_element_type=f32)
            b = None
            for c in range(F // FC):
                hh = jnp.dot(xb, w1_ref[:, c * FC:(c + 1) * FC], preferred_element_type=f32)
                hh = hh + b1_ref[:, c * FC:(c + 1) * FC].astype(f32)
                act = _mish(hh).astype(bf16)
                d = jnp.dot(act, w2_ref[c * FC:(c + 1) * FC, :], preferred_element_type=f32)
                b = d if b is None else b + d
            g = jnp.tile(g_s[pl.ds(r, FB), :], (1, D // 128))
            o_ref[pl.ds(r, FB), :] = (g * a + (1.0 - g) * b).astype(o_ref.dtype)
            return 0
        lax.fori_loop(0, S // FB, tail, 0)

    return kernel


_kernel = make_kernel()


@jax.jit
def pallas_gated_mix__mha_block__dense_activation_mish__prompt_kernel(
    A_x, A_wqkv, A_wo, B_x, B_w1, B_b1, B_w2, gate_w
):
    del B_x
    out = pl.pallas_call(
        _kernel,
        out_shape=jax.ShapeDtypeStruct((S, D), bf16),
        scratch_shapes=[
            pltpu.VMEM((DP + D, D), bf16),
            pltpu.VMEM((D, DP), bf16),
            pltpu.VMEM((S, DP), bf16),
            pltpu.VMEM((DP, S), bf16),
            pltpu.VMEM((D, S), f32),
            pltpu.VMEM((D, S), f32),
            pltpu.VMEM((S, 128), f32),
        ],
        compiler_params=pltpu.CompilerParams(vmem_limit_bytes=110 * 1024 * 1024),
        name="gated_mix",
    )(A_x.reshape(S, D), A_wqkv, A_wo, B_w1, B_b1.reshape(1, F), B_w2, gate_w.reshape(1, D))
    return out.reshape(1, S, D)
```

```python
import math

import jax
import jax.numpy as jnp
from jax import lax
import jax.experimental.pallas as pl
import jax.experimental.pallas.tpu as pltpu

bf16 = jnp.bfloat16
f32 = jnp.float32

S, D, H, DH, F = 2048, 640, 32, 20, 1536
HPT = 6
NT = (H + HPT - 1) // HPT
DP = NT * 128
GATE_LANE = HPT * DH
QSCALE = (DH ** -0.5) * math.log2(math.e)
L_LO, L_HI = 2.0 ** -60, 2.0 ** 60


def _pad_tile(w_ref, t):
    lo = t * HPT * DH
    hi = min(lo + HPT * DH, D)
    return jnp.concatenate(
        [w_ref[:, lo:hi], jnp.zeros((D, 128 - (hi - lo)), bf16)], axis=1)


def _mish(h):
    e = jnp.exp(jnp.minimum(h, 20.0))
    n = e * (e + 2.0)
    return h * (n / (n + 2.0))


def make_kernel(TQ=512, KB=256, QB=2048, DEPTH=2, RING=True, PB=512, FB=512, FC=512, PH='wpat'):
    NQB = S // QB
    R = DEPTH + 1
    NPB = S // PB
    NFB = S // FB

    def kernel(x_hbm, wqkv_hbm, wo_hbm, w1_hbm, b1_hbm, w2_hbm, gw_hbm, o_hbm,
               x_s, wq_s, wkr_s, wv_s, wo_s, w1_s, b1_s, w2_s, gw_s,
               wqvT_s, wk_s, k_s, qT_s, vT_s, oT_s, g_s, p_s, o_s, sems, osems):
        def cp(src, dst, i):
            return pltpu.make_async_copy(src, dst, sems.at[i])
        xc = [cp(x_hbm.at[pl.ds(i * PB, PB), :], x_s.at[pl.ds(i * PB, PB), :], i) for i in range(NPB)]
        n0 = NPB
        c_wk = cp(wqkv_hbm.at[:, pl.ds(D, D)], wkr_s, n0)
        c_gw = cp(gw_hbm, gw_s, n0 + 1)
        c_wq = cp(wqkv_hbm.at[:, pl.ds(0, D)], wq_s, n0 + 2)
        c_wv = cp(wqkv_hbm.at[:, pl.ds(2 * D, D)], wv_s, n0 + 3)
        c_w1 = cp(w1_hbm, w1_s, n0 + 4)
        c_b1 = cp(b1_hbm, b1_s, n0 + 5)
        c_w2 = cp(w2_hbm, w2_s, n0 + 6)
        c_wo = cp(wo_hbm, wo_s, n0 + 7)

        c_wk.start()
        c_gw.start()
        xc[0].start()
        oT_s[...] = jnp.zeros_like(oT_s)
        c_wk.wait()
        c_gw.wait()
        for i in range(1, NPB):
            xc[i].start()
        gcol = jnp.broadcast_to(gw_s[...], (128, D)).T
        lane = lax.broadcasted_iota(jnp.int32, (D, 128), 1)
        wk_s[:, 0:128] = jnp.where(lane == GATE_LANE, gcol, _pad_tile(wkr_s, 0))
        for t in range(1, NT):
            wk_s[:, t * 128:(t + 1) * 128] = _pad_tile(wkr_s, t)

        def kproj(r):
            xb = x_s[pl.ds(r, PB), :]
            kk = jnp.dot(xb, wk_s[...], preferred_element_type=f32)
            k_s[pl.ds(r, PB), :] = kk.astype(bf16)
            g = jax.nn.sigmoid(kk[:, GATE_LANE:GATE_LANE + 1])
            g_s[pl.ds(r, PB), :] = jnp.broadcast_to(g, (PB, 128))

        xc[0].wait()
        c_wq.start()
        c_wv.start()
        for i in range(NPB):
            if i > 0:
                xc[i].wait()
            if i == NPB - 1:
                c_wq.wait()
                c_wv.wait()
                c_w1.start()
                c_b1.start()
                c_w2.start()
                c_wo.start()
                for t in range(NT):
                    wqvT_s[t * 128:(t + 1) * 128, :] = _pad_tile(wq_s, t).T
                wqvT_s[DP:DP + D, :] = wv_s[...].T
            kproj(i * PB)

        def proj(i, _):
            r = pl.multiple_of(i * PB, PB)
            xb = x_s[pl.ds(r, PB), :]
            qv = lax.dot_general(wqvT_s[...], xb, (((1,), (1,)), ((), ())),
                                 preferred_element_type=f32)
            qT_s[:, pl.ds(r, PB)] = (qv[0:DP] * QSCALE).astype(bf16)
            vT_s[:, pl.ds(r, PB)] = qv[DP:DP + D].astype(bf16).astype(f32)
            return 0
        lax.fori_loop(0, NPB if 'p' in PH else 0, proj, 0)

        def head_ctx(h, width):
            t = pl.multiple_of((h // HPT) * 128, 128)
            lo = (h % HPT) * DH
            odd = h % 2
            vo = pl.multiple_of((h // 2) * 40 + odd * 16, 8)
            ri = lax.broadcasted_iota(jnp.int32, (128, TQ), 0)
            qm = (ri >= lo) & (ri < lo + DH)
            wr = lax.broadcasted_iota(jnp.int32, (24, width), 0)
            valid = (wr >= odd * 4) & (wr < odd * 4 + DH)
            wr2 = lax.broadcasted_iota(jnp.int32, (24, TQ), 0)
            valid2 = (wr2 >= odd * 4) & (wr2 < odd * 4 + DH)
            return t, vo, qm, valid, valid2

        def finish(acc, valid2, vo, qo):
            l = jnp.max(jnp.where(valid2, 0.0, acc), axis=0, keepdims=True)
            o = acc / l
            sl = (pl.ds(vo, 24), pl.ds(qo, TQ))
            oT_s[sl] = jnp.where(valid2, o, oT_s[sl])
            return l

        def attn_fast(it, bad):
            h = it // NQB
            qo = pl.multiple_of((it % NQB) * QB, QB)
            t, vo, qm, valid, valid2 = head_ctx(h, KB)
            nk = S // KB
            steps = [(a, b) for a in range(QB // TQ) for b in range(nk)]
            qs, ps, accs = {}, {}, {}
            flags = [bad]

            def pv(s):
                a, b = steps[s]
                v = jnp.where(valid, vT_s[pl.ds(vo, 24), b * KB:(b + 1) * KB], 1.0)
                p = p_s[s % R] if RING else ps.pop(s)
                d = lax.dot_general(v, p, (((1,), (0,)), ((), ())), preferred_element_type=f32)
                accs[a] = d if b == 0 else accs[a] + d
                if b == nk - 1:
                    l = finish(accs.pop(a), valid2, vo, qo + a * TQ)
                    ok = (l >= L_LO) & (l <= L_HI)
                    flags[0] = jnp.maximum(flags[0], jnp.where(ok, 0.0, 1.0))
            for s, (a, b) in enumerate(steps):
                if b == 0:
                    q = qT_s[pl.ds(t, 128), pl.ds(qo + a * TQ, TQ)]
                    qs[a] = jnp.where(qm, q, jnp.zeros_like(q))
                st = jnp.dot(k_s[b * KB:(b + 1) * KB, pl.ds(t, 128)], qs[a],
                             preferred_element_type=f32)
                if s >= DEPTH:
                    pv(s - DEPTH)
                p = jnp.exp2(st).astype(bf16)
                if RING:
                    p_s[s % R] = p
                else:
                    ps[s] = p
            for s in range(len(steps) - DEPTH, len(steps)):
                pv(s)
            return flags[0]
        bad = lax.fori_loop(0, H * NQB if 'a' in PH else 0, attn_fast, jnp.zeros((1, TQ), f32))

        @pl.when(jnp.max(bad) > 0.0)
        def _safe():
            SB = 256

            def attn_safe(it, _):
                h = it // (S // TQ)
                qo = pl.multiple_of((it % (S // TQ)) * TQ, TQ)
                t, vo, qm, valid, valid2 = head_ctx(h, SB)
                q = qT_s[pl.ds(t, 128), pl.ds(qo, TQ)]
                q = jnp.where(qm, q, jnp.zeros_like(q))

                def mx(i, m):
                    r = pl.multiple_of(i * SB, SB)
                    st = jnp.dot(k_s[pl.ds(r, SB), pl.ds(t, 128)], q, preferred_element_type=f32)
                    return jnp.maximum(m, jnp.max(st, axis=0, keepdims=True))
                m = lax.fori_loop(0, S // SB, mx, jnp.full((1, TQ), -jnp.inf, f32))

                def ex(i, acc):
                    r = pl.multiple_of(i * SB, SB)
                    st = jnp.dot(k_s[pl.ds(r, SB), pl.ds(t, 128)], q, preferred_element_type=f32)
                    p = jnp.exp2(st - m).astype(bf16)
                    v = jnp.where(valid, vT_s[pl.ds(vo, 24), pl.ds(r, SB)], 1.0)
                    return acc + lax.dot_general(v, p, (((1,), (0,)), ((), ())),
                                                 preferred_element_type=f32)
                acc = lax.fori_loop(0, S // SB, ex, jnp.zeros((24, TQ), f32))
                finish(acc, valid2, vo, qo)
                return 0
            lax.fori_loop(0, H * (S // TQ), attn_safe, 0)

        c_w1.wait()
        c_b1.wait()
        c_w2.wait()
        c_wo.wait()

        def ocp(i, slot):
            return pltpu.make_async_copy(o_s.at[slot], o_hbm.at[pl.ds(i * FB, FB), :], osems.at[slot])

        def tail(i, _):
            r = pl.multiple_of(i * FB, FB)
            slot = i % 2
            xb = x_s[pl.ds(r, FB), :]
            ot = oT_s[:, pl.ds(r, FB)].astype(bf16)
            a = lax.dot_general(ot, wo_s[...], (((0,), (0,)), ((), ())),
                                preferred_element_type=f32)
            b = None
            for c in range(F // FC):
                hh = jnp.dot(xb, w1_s[:, c * FC:(c + 1) * FC], preferred_element_type=f32)
                hh = hh + b1_s[:, c * FC:(c + 1) * FC].astype(f32)
                act = _mish(hh).astype(bf16)
                d = jnp.dot(act, w2_s[c * FC:(c + 1) * FC, :], preferred_element_type=f32)
                b = d if b is None else b + d
            g = jnp.tile(g_s[pl.ds(r, FB), :], (1, D // 128))
            res = (g * a + (1.0 - g) * b).astype(bf16)

            @pl.when(i >= 2)
            def _():
                ocp(i - 2, slot).wait()
            o_s[slot] = res
            ocp(i, slot).start()
            return 0
        lax.fori_loop(0, NFB, tail, 0)
        ocp(NFB - 2, NFB % 2).wait()
        ocp(NFB - 1, (NFB - 1) % 2).wait()

    scratch = [
        pltpu.VMEM((S, D), bf16),
        pltpu.VMEM((D, D), bf16),
        pltpu.VMEM((D, D), bf16),
        pltpu.VMEM((D, D), bf16),
        pltpu.VMEM((D, D), bf16),
        pltpu.VMEM((D, F), bf16),
        pltpu.VMEM((1, F), bf16),
        pltpu.VMEM((F, D), bf16),
        pltpu.VMEM((1, D), bf16),
        pltpu.VMEM((DP + D, D), bf16),
        pltpu.VMEM((D, DP), bf16),
        pltpu.VMEM((S, DP), bf16),
        pltpu.VMEM((DP, S), bf16),
        pltpu.VMEM((D, S), f32),
        pltpu.VMEM((D, S), f32),
        pltpu.VMEM((S, 128), f32),
        pltpu.VMEM((R, KB, TQ), bf16),
        pltpu.VMEM((2, FB, D), bf16),
        pltpu.SemaphoreType.DMA((NPB + 8,)),
        pltpu.SemaphoreType.DMA((2,)),
    ]
    return kernel, scratch


_kernel, _scratch = make_kernel()


@jax.jit
def pallas_gated_mix__mha_block__dense_activation_mish__prompt_kernel(
    A_x, A_wqkv, A_wo, B_x, B_w1, B_b1, B_w2, gate_w
):
    del B_x
    any_spec = pl.BlockSpec(memory_space=pl.ANY)
    out = pl.pallas_call(
        _kernel,
        out_shape=jax.ShapeDtypeStruct((S, D), bf16),
        in_specs=[any_spec] * 7,
        out_specs=any_spec,
        scratch_shapes=_scratch,
        compiler_params=pltpu.CompilerParams(vmem_limit_bytes=110 * 1024 * 1024),
        name="gated_mix",
    )(A_x.reshape(S, D), A_wqkv, A_wo, B_w1, B_b1.reshape(1, F), B_w2, gate_w.reshape(1, D))
    return out.reshape(1, S, D)
```

```python
import math

import jax
import jax.numpy as jnp
from jax import lax
import jax.experimental.pallas as pl
import jax.experimental.pallas.tpu as pltpu

bf16 = jnp.bfloat16
f32 = jnp.float32

S, D, H, DH, F = 2048, 640, 32, 20, 1536
HPT = 6
NT = (H + HPT - 1) // HPT
DP = NT * 128
QSCALE = (DH ** -0.5) * math.log2(math.e)
L_LO, L_HI = 2.0 ** -60, 2.0 ** 60
F32_BIG = 3.0e38


def _mish(h):
    e = jnp.exp(jnp.minimum(h, 20.0))
    n = e * (e + 2.0)
    return h * (n / (n + 2.0))


def make_kernel(TQ=512, KB=256, HB=4, DEPTH=4, RING=True, PB=512, FB=256, FC=512, PH='wpat'):
    R = DEPTH + 1
    NPB = S // PB
    NFB = S // FB

    def kernel(x_hbm, wqkv_hbm, wo_hbm, w1_hbm, b1_hbm, w2_hbm, gw_hbm, o_hbm,
               x_s, wq_s, wkr_s, wv_s, wo_s, w1_s, b1_s, w2_s, gw_s,
               wqvT_s, k_s, qT_s, vT_s, oT_s, p_s, o_s, sems, osems):
        def cp(src, dst, i):
            return pltpu.make_async_copy(src, dst, sems.at[i])
        xc = [cp(x_hbm.at[pl.ds(i * PB, PB), :], x_s.at[pl.ds(i * PB, PB), :], i) for i in range(NPB)]
        n0 = NPB
        c_wk = cp(wqkv_hbm.at[:, pl.ds(D, D)], wkr_s, n0)
        c_gw = cp(gw_hbm, gw_s, n0 + 1)
        c_wq = cp(wqkv_hbm.at[:, pl.ds(0, D)], wq_s, n0 + 2)
        c_wv = cp(wqkv_hbm.at[:, pl.ds(2 * D, D)], wv_s, n0 + 3)
        c_w1 = cp(w1_hbm, w1_s, n0 + 4)
        c_b1 = cp(b1_hbm, b1_s, n0 + 5)
        c_w2 = cp(w2_hbm, w2_s, n0 + 6)
        c_wo = cp(wo_hbm, wo_s, n0 + 7)

        c_wk.start()
        xc[0].start()
        oT_s[...] = jnp.zeros_like(oT_s)
        c_wk.wait()
        for i in range(1, NPB):
            xc[i].start()
        def kproj(r):
            xb = x_s[pl.ds(r, PB), :]
            kk = jnp.dot(xb, wkr_s[...], preferred_element_type=f32).astype(bf16)
            for t in range(NT):
                lo = t * HPT * DH
                hi = min(lo + HPT * DH, D)
                k_s[pl.ds(r, PB), t * 128:(t + 1) * 128] = jnp.concatenate(
                    [kk[:, lo:hi], jnp.zeros((PB, 128 - (hi - lo)), bf16)], axis=1)

        xc[0].wait()
        c_wq.start()
        c_wv.start()

        def kloop(i, _):
            r = pl.multiple_of(i * PB, PB)

            @pl.when(i > 0)
            def _():
                cp(x_hbm.at[pl.ds(r, PB), :], x_s.at[pl.ds(r, PB), :], i).wait()
            kproj(r)
            return 0
        lax.fori_loop(0, NPB - 1, kloop, 0)
        xc[NPB - 1].wait()
        c_wq.wait()
        c_wv.wait()
        c_gw.start()
        c_w1.start()
        c_b1.start()
        c_w2.start()
        c_wo.start()
        wqvT_s[0:D, :] = wq_s[...].T
        wqvT_s[D:2 * D, :] = wv_s[...].T
        kproj((NPB - 1) * PB)

        def proj(i, _):
            r = pl.multiple_of(i * PB, PB)
            xb = x_s[pl.ds(r, PB), :]
            qv = lax.dot_general(wqvT_s[...], xb, (((1,), (1,)), ((), ())),
                                 preferred_element_type=f32)
            for t in range(NT):
                lo = t * HPT * DH
                hi = min(lo + HPT * DH, D)
                qt = jnp.concatenate([qv[lo:hi] * QSCALE, jnp.zeros((128 - (hi - lo), PB), f32)], axis=0)
                qT_s[t * 128:(t + 1) * 128, pl.ds(r, PB)] = qt.astype(bf16)
            vT_s[:, pl.ds(r, PB)] = qv[D:2 * D].astype(bf16).astype(f32)
            return 0
        lax.fori_loop(0, NPB if 'p' in PH else 0, proj, 0)

        def head_ctx(h, odd, width):
            t = pl.multiple_of((h // HPT) * 128, 128)
            lo = (h % HPT) * DH
            vo = pl.multiple_of((h // 2) * 40 + odd * 16, 8)
            ri = lax.broadcasted_iota(jnp.int32, (128, TQ), 0)
            qm = (ri >= lo) & (ri < lo + DH)
            wr = lax.broadcasted_iota(jnp.int32, (24, width), 0)
            valid = (wr >= odd * 4) & (wr < odd * 4 + DH)
            wr2 = lax.broadcasted_iota(jnp.int32, (24, TQ), 0)
            valid2 = (wr2 >= odd * 4) & (wr2 < odd * 4 + DH)
            return t, vo, qm, valid, valid2

        def finish(acc, valid2, vo, qo):
            l = jnp.max(jnp.where(valid2, 0.0, acc), axis=0, keepdims=True)
            o = acc / l
            sl = (pl.ds(vo, 24), pl.ds(qo, TQ))
            oT_s[sl] = jnp.where(valid2, o, oT_s[sl])
            return l, o

        def attn_fast(it, bad):
            ctx = [head_ctx(it * HB + j, j % 2, KB) for j in range(HB)]
            nk = S // KB
            steps = [(j, a, b) for j in range(HB) for a in range(S // TQ) for b in range(nk)]
            qs, ps, accs = {}, {}, {}
            flags = [bad]

            def pv(s):
                j, a, b = steps[s]
                t, vo, qm, valid, valid2 = ctx[j]
                v = jnp.where(valid, vT_s[pl.ds(vo, 24), b * KB:(b + 1) * KB], 1.0)
                p = p_s[s % R] if RING else ps.pop(s)
                d = lax.dot_general(v, p, (((1,), (0,)), ((), ())), preferred_element_type=f32)
                accs[j, a] = d if b == 0 else accs[j, a] + d
                if b == nk - 1:
                    l, o = finish(accs.pop((j, a)), valid2, vo, a * TQ)
                    ok = (l >= L_LO) & (l <= L_HI) & (jnp.max(jnp.abs(o), axis=0, keepdims=True) < F32_BIG)
                    flags[0] = jnp.maximum(flags[0], jnp.where(ok, 0.0, 1.0))
            for s, (j, a, b) in enumerate(steps):
                t, vo, qm, valid, valid2 = ctx[j]
                if b == 0:
                    q = qT_s[pl.ds(t, 128), a * TQ:(a + 1) * TQ]
                    qs[j, a] = jnp.where(qm, q, jnp.zeros_like(q))
                st = jnp.dot(k_s[b * KB:(b + 1) * KB, pl.ds(t, 128)], qs[j, a],
                             preferred_element_type=f32)
                if s >= DEPTH:
                    pv(s - DEPTH)
                p = jnp.exp2(st).astype(bf16)
                if RING:
                    p_s[s % R] = p
                else:
                    ps[s] = p
            for s in range(len(steps) - DEPTH, len(steps)):
                pv(s)
            return flags[0]
        bad = lax.fori_loop(0, H // HB if 'a' in PH else 0, attn_fast, jnp.zeros((1, TQ), f32))

        @pl.when(jnp.max(bad) > 0.0)
        def _safe():
            SB = 256

            def attn_safe(it, _):
                h = it // (S // TQ)
                qo = pl.multiple_of((it % (S // TQ)) * TQ, TQ)
                t, vo, qm, valid, valid2 = head_ctx(h, h % 2, SB)
                q = qT_s[pl.ds(t, 128), pl.ds(qo, TQ)]
                q = jnp.where(qm, q, jnp.zeros_like(q))

                def mx(i, m):
                    r = pl.multiple_of(i * SB, SB)
                    st = jnp.dot(k_s[pl.ds(r, SB), pl.ds(t, 128)], q, preferred_element_type=f32)
                    return jnp.maximum(m, jnp.max(st, axis=0, keepdims=True))
                m = lax.fori_loop(0, S // SB, mx, jnp.full((1, TQ), -jnp.inf, f32))

                def ex(i, acc):
                    r = pl.multiple_of(i * SB, SB)
                    st = jnp.dot(k_s[pl.ds(r, SB), pl.ds(t, 128)], q, preferred_element_type=f32)
                    p = jnp.exp2(st - m).astype(bf16)
                    v = jnp.where(valid, vT_s[pl.ds(vo, 24), pl.ds(r, SB)], 1.0)
                    return acc + lax.dot_general(v, p, (((1,), (0,)), ((), ())),
                                                 preferred_element_type=f32)
                acc = lax.fori_loop(0, S // SB, ex, jnp.zeros((24, TQ), f32))
                finish(acc, valid2, vo, qo)
                return 0
            lax.fori_loop(0, H * (S // TQ), attn_safe, 0)

        c_gw.wait()
        c_w1.wait()
        c_b1.wait()
        c_w2.wait()
        c_wo.wait()

        def ocp(i, slot):
            return pltpu.make_async_copy(o_s.at[slot], o_hbm.at[pl.ds(i * FB, FB), :], osems.at[slot])

        def tail(i, _):
            r = pl.multiple_of(i * FB, FB)
            slot = i % 2
            xb = x_s[pl.ds(r, FB), :]
            b1 = b1_s[...].astype(f32).reshape(1, F)
            gw = gw_s[...].astype(f32).reshape(1, D)
            ot = oT_s[:, pl.ds(r, FB)].astype(bf16)
            a = lax.dot_general(ot, wo_s[...], (((0,), (0,)), ((), ())),
                                preferred_element_type=f32)
            b = None
            for c in range(F // FC):
                hh = jnp.dot(xb, w1_s[:, c * FC:(c + 1) * FC], preferred_element_type=f32)
                hh = hh + b1[:, c * FC:(c + 1) * FC]
                act = _mish(hh).astype(bf16)
                d = jnp.dot(act, w2_s[c * FC:(c + 1) * FC, :], preferred_element_type=f32)
                b = d if b is None else b + d
            gl = jnp.sum(xb.astype(f32) * gw, axis=1, keepdims=True)
            g = jax.nn.sigmoid(gl)
            res = (g * a + (1.0 - g) * b).astype(bf16)

            @pl.when(i >= 2)
            def _():
                ocp(i - 2, slot).wait()
            o_s[slot] = res
            ocp(i, slot).start()
            return 0
        lax.fori_loop(0, NFB, tail, 0)
        ocp(NFB - 2, NFB % 2).wait()
        ocp(NFB - 1, (NFB - 1) % 2).wait()

    scratch = [
        pltpu.VMEM((S, D), bf16),
        pltpu.VMEM((D, D), bf16),
        pltpu.VMEM((D, D), bf16),
        pltpu.VMEM((D, D), bf16),
        pltpu.VMEM((D, D), bf16),
        pltpu.VMEM((D, F), bf16),
        pltpu.VMEM((F,), bf16),
        pltpu.VMEM((F, D), bf16),
        pltpu.VMEM((D,), bf16),
        pltpu.VMEM((2 * D, D), bf16),
        pltpu.VMEM((S, DP), bf16),
        pltpu.VMEM((DP, S), bf16),
        pltpu.VMEM((D, S), f32),
        pltpu.VMEM((D, S), f32),
        pltpu.VMEM((R, KB, TQ), bf16),
        pltpu.VMEM((2, FB, D), bf16),
        pltpu.SemaphoreType.DMA((NPB + 8,)),
        pltpu.SemaphoreType.DMA((2,)),
    ]
    return kernel, scratch


_kernel, _scratch = make_kernel()


@jax.jit
def pallas_gated_mix__mha_block__dense_activation_mish__prompt_kernel(
    A_x, A_wqkv, A_wo, B_x, B_w1, B_b1, B_w2, gate_w
):
    del B_x
    any_spec = pl.BlockSpec(memory_space=pl.ANY)
    out = pl.pallas_call(
        _kernel,
        out_shape=jax.ShapeDtypeStruct((S, D), bf16),
        in_specs=[any_spec] * 7,
        out_specs=any_spec,
        scratch_shapes=_scratch,
        compiler_params=pltpu.CompilerParams(vmem_limit_bytes=110 * 1024 * 1024),
        name="gated_mix",
    )(A_x.reshape(S, D), A_wqkv, A_wo, B_w1, B_b1, B_w2, gate_w)
    return out.reshape(1, S, D)
```

```python
import math

import jax
import jax.numpy as jnp
from jax import lax
import jax.experimental.pallas as pl
import jax.experimental.pallas.tpu as pltpu

bf16 = jnp.bfloat16
f32 = jnp.float32

S, D, H, DH, F = 2048, 640, 32, 20, 1536
HPT = 4
HP = 128 // HPT
NT = H // HPT
VW = 24
QSCALE = (DH ** -0.5) * math.log2(math.e)
L_LO, L_HI, F32_BIG = 2.0 ** -60, 2.0 ** 60, 3.0e38

PB = 512
TQ = 512
KB = 256
HB = HPT
DEPTH = 4
FB = 256
FC = 512
NPB, NFB = S // PB, S // FB

_NT = (((1,), (1,)), ((), ()))
_NN = (((1,), (0,)), ((), ()))
_TN = (((0,), (0,)), ((), ()))


def _dot(a, b, dims=_NN):
    return lax.dot_general(a, b, dims, preferred_element_type=f32)


def _mish(h):
    e = jnp.exp(jnp.minimum(h, 20.0))
    n = e * (e + 2.0)
    return h * (n / (n + 2.0))


def _kernel(x_hbm, wqkv_hbm, wo_hbm, w1_hbm, b1_hbm, w2_hbm, gw_hbm, o_hbm,
            x_s, wq_s, wk_s, wv_s, wo_s, w1_s, b1_s, w2_s, gw_s,
            wkT_s, wqvT_s, k_s, qT_s, vT_s, oT_s, p_s, o_s, sems, osems):
    def cp(src, dst, i):
        return pltpu.make_async_copy(src, dst, sems.at[i])

    def x_copy(i):
        rows = pl.ds(pl.multiple_of(i * PB, PB), PB)
        return cp(x_hbm.at[rows, :], x_s.at[rows, :], i)

    c_wq = cp(wqkv_hbm.at[:, pl.ds(0, D)], wq_s, NPB)
    c_wk = cp(wqkv_hbm.at[:, pl.ds(D, D)], wk_s, NPB + 1)
    c_wv = cp(wqkv_hbm.at[:, pl.ds(2 * D, D)], wv_s, NPB + 2)
    late = [cp(gw_hbm, gw_s, NPB + 3), cp(w1_hbm, w1_s, NPB + 4), cp(b1_hbm, b1_s, NPB + 5),
            cp(w2_hbm, w2_s, NPB + 6), cp(wo_hbm, wo_s, NPB + 7)]

    c_wk.start()
    x_copy(0).start()
    oT_s[...] = jnp.zeros_like(oT_s)
    c_wk.wait()
    for i in range(1, NPB):
        x_copy(i).start()
    wkT_s[...] = wk_s[...].T

    def kproj(r):
        kT = _dot(wkT_s[...], x_s[pl.ds(r, PB), :], _NT)
        z = jnp.zeros((HP - DH, PB), f32)
        for t in range(NT):
            parts = []
            for h in range(t * HPT, (t + 1) * HPT):
                parts += [kT[h * DH:(h + 1) * DH], z]
            tile = jnp.concatenate(parts, axis=0).astype(bf16)
            k_s[pl.ds(r, PB), t * 128:(t + 1) * 128] = tile.T

    x_copy(0).wait()
    c_wq.start()
    c_wv.start()

    def kloop(i, _):
        @pl.when(i > 0)
        def _():
            x_copy(i).wait()
        kproj(pl.multiple_of(i * PB, PB))
        return 0
    lax.fori_loop(0, NPB - 1, kloop, 0)
    x_copy(NPB - 1).wait()
    c_wq.wait()
    c_wv.wait()
    for c in late:
        c.start()
    wqvT_s[0:D, :] = wq_s[...].T
    wqvT_s[D:2 * D, :] = wv_s[...].T
    kproj((NPB - 1) * PB)

    def qvproj(i, _):
        r = pl.multiple_of(i * PB, PB)
        qv = _dot(wqvT_s[...], x_s[pl.ds(r, PB), :], _NT)
        qsc = qv[0:D] * QSCALE
        z = jnp.zeros((HP - DH, PB), f32)
        for h in range(H):
            qt = jnp.concatenate([qsc[h * DH:(h + 1) * DH], z], axis=0)
            qT_s[h * HP:(h + 1) * HP, pl.ds(r, PB)] = qt.astype(bf16)
        vT_s[:, pl.ds(r, PB)] = qv[D:2 * D].astype(bf16).astype(f32)
        return 0
    lax.fori_loop(0, NPB, qvproj, 0)

    def head_ctx(h, odd, width):
        t = pl.multiple_of((h // HPT) * 128, 128)
        vo = pl.multiple_of((h // 2) * 2 * DH + odd * 16, 8)

        def rows_ok(n):
            wr = lax.broadcasted_iota(jnp.int32, (VW, n), 0)
            return (wr >= odd * 4) & (wr < odd * 4 + DH)
        return t, vo, rows_ok(width), rows_ok(TQ)

    def pv_dot(vo, valid, keys, p):
        v = jnp.where(valid, vT_s[pl.ds(vo, VW), keys], 1.0)
        return _dot(v, p)

    def finish(acc, valid, vo, qo):
        l = jnp.max(jnp.where(valid, 0.0, acc), axis=0, keepdims=True)
        o = acc / l
        sl = (pl.ds(vo, VW), pl.ds(qo, TQ))
        oT_s[sl] = jnp.where(valid, o, oT_s[sl])
        return l, o

    def attn_fast(it, bad):
        ctx = [head_ctx(it * HB + j, j % 2, KB) for j in range(HB)]
        nk = S // KB
        steps = [(j, a, b) for j in range(HB) for a in range(S // TQ) for b in range(nk)]
        qs, accs, flags = {}, {}, [bad]

        def pv(s):
            j, a, b = steps[s]
            _, vo, valid_k, valid_q = ctx[j]
            d = pv_dot(vo, valid_k, slice(b * KB, (b + 1) * KB), p_s[s % (DEPTH + 1)])
            accs[j, a] = d if b == 0 else accs[j, a] + d
            if b == nk - 1:
                l, o = finish(accs.pop((j, a)), valid_q, vo, a * TQ)
                ok = ((l >= L_LO) & (l <= L_HI)
                      & (jnp.max(jnp.abs(o), axis=0, keepdims=True) < F32_BIG))
                flags[0] = jnp.maximum(flags[0], jnp.where(ok, 0.0, 1.0))

        for s, (j, a, b) in enumerate(steps):
            t = ctx[j][0]
            if b == 0:
                q = qT_s[pl.ds(t + j * HP, HP), a * TQ:(a + 1) * TQ]
                if j:
                    q = jnp.concatenate([jnp.zeros((j * HP, TQ), bf16), q], axis=0)
                qs[j, a] = q
            kt = k_s[b * KB:(b + 1) * KB, pl.ds(t, 128)][:, :HP * (j + 1)]
            st = _dot(kt, qs[j, a])
            if s >= DEPTH:
                pv(s - DEPTH)
            p_s[s % (DEPTH + 1)] = jnp.exp2(st).astype(bf16)
        for s in range(len(steps) - DEPTH, len(steps)):
            pv(s)
        return flags[0]
    bad = lax.fori_loop(0, H // HB, attn_fast, jnp.zeros((1, TQ), f32))

    @pl.when(jnp.max(bad) > 0.0)
    def _attn_with_true_max():
        def attn_safe(it, _):
            h = it // (S // TQ)
            qo = pl.multiple_of((it % (S // TQ)) * TQ, TQ)
            t, vo, valid_k, valid_q = head_ctx(h, h % 2, KB)
            lo = (h % HPT) * HP
            ri = lax.broadcasted_iota(jnp.int32, (128, TQ), 0)
            q = qT_s[pl.ds(t, 128), pl.ds(qo, TQ)]
            q = jnp.where((ri >= lo) & (ri < lo + DH), q, jnp.zeros_like(q))

            def scores(r):
                return _dot(k_s[pl.ds(r, KB), pl.ds(t, 128)], q)

            def row_max(i, m):
                st = scores(pl.multiple_of(i * KB, KB))
                return jnp.maximum(m, jnp.max(st, axis=0, keepdims=True))
            m = lax.fori_loop(0, S // KB, row_max, jnp.full((1, TQ), -jnp.inf, f32))

            def accumulate(i, acc):
                r = pl.multiple_of(i * KB, KB)
                p = jnp.exp2(scores(r) - m).astype(bf16)
                return acc + pv_dot(vo, valid_k, pl.ds(r, KB), p)
            acc = lax.fori_loop(0, S // KB, accumulate, jnp.zeros((VW, TQ), f32))
            finish(acc, valid_q, vo, qo)
            return 0
        lax.fori_loop(0, H * (S // TQ), attn_safe, 0)

    for c in late:
        c.wait()

    def o_copy(i, slot):
        return pltpu.make_async_copy(o_s.at[slot], o_hbm.at[pl.ds(i * FB, FB), :], osems.at[slot])

    def tail(i, _):
        r = pl.multiple_of(i * FB, FB)
        slot = i % 2
        xb = x_s[pl.ds(r, FB), :]
        b1 = b1_s[...].astype(f32).reshape(1, F)
        gw = gw_s[...].astype(f32).reshape(1, D)

        def hidden(c):
            cols = slice(c * FC, (c + 1) * FC)
            return _mish(_dot(xb, w1_s[:, cols]) + b1[:, cols]).astype(bf16)

        act, b = hidden(0), None
        for c in range(F // FC):
            nxt = hidden(c + 1) if c + 1 < F // FC else None
            d = _dot(act, w2_s[c * FC:(c + 1) * FC, :])
            b = d if b is None else b + d
            act = nxt
        a = _dot(oT_s[:, pl.ds(r, FB)].astype(bf16), wo_s[...], _TN)
        g = jax.nn.sigmoid(jnp.sum(xb.astype(f32) * gw, axis=1, keepdims=True))
        res = (g * a + (1.0 - g) * b).astype(bf16)

        @pl.when(i >= 2)
        def _():
            o_copy(i - 2, slot).wait()
        o_s[slot] = res
        o_copy(i, slot).start()
        return 0
    lax.fori_loop(0, NFB, tail, 0)
    o_copy(NFB - 2, NFB % 2).wait()
    o_copy(NFB - 1, (NFB - 1) % 2).wait()


@jax.jit
def pallas_gated_mix__mha_block__dense_activation_mish__prompt_kernel(
    A_x: jax.Array,
    A_wqkv: jax.Array,
    A_wo: jax.Array,
    B_x: jax.Array,
    B_w1: jax.Array,
    B_b1: jax.Array,
    B_w2: jax.Array,
    gate_w: jax.Array,
):
    del B_x
    hbm = pl.BlockSpec(memory_space=pl.ANY)
    out = pl.pallas_call(
        _kernel,
        out_shape=jax.ShapeDtypeStruct((S, D), bf16),
        in_specs=[hbm] * 7,
        out_specs=hbm,
        scratch_shapes=[
            pltpu.VMEM((S, D), bf16),
            pltpu.VMEM((D, D), bf16),
            pltpu.VMEM((D, D), bf16),
            pltpu.VMEM((D, D), bf16),
            pltpu.VMEM((D, D), bf16),
            pltpu.VMEM((D, F), bf16),
            pltpu.VMEM((F,), bf16),
            pltpu.VMEM((F, D), bf16),
            pltpu.VMEM((D,), bf16),
            pltpu.VMEM((D, D), bf16),
            pltpu.VMEM((2 * D, D), bf16),
            pltpu.VMEM((S, NT * 128), bf16),
            pltpu.VMEM((NT * 128, S), bf16),
            pltpu.VMEM((D, S), f32),
            pltpu.VMEM((D, S), f32),
            pltpu.VMEM((DEPTH + 1, KB, TQ), bf16),
            pltpu.VMEM((2, FB, D), bf16),
            pltpu.SemaphoreType.DMA((NPB + 8,)),
            pltpu.SemaphoreType.DMA((2,)),
        ],
        compiler_params=pltpu.CompilerParams(vmem_limit_bytes=100 * 1024 * 1024),
        name="gated_mix",
    )(A_x.reshape(S, D), A_wqkv, A_wo, B_w1, B_b1, B_w2, gate_w)
    return out.reshape(1, S, D)
```
